```python
import os as _os
_os.environ.setdefault("JAX_PLATFORMS", "cpu")
import jax
import jax.numpy as jnp

def _softmax(x, axis=-1):
    return jax.nn.softmax(x, axis=axis)
def _gelu(x):
    return jax.nn.gelu(x, approximate=True)
def _silu(x):
    return jax.nn.silu(x)
def _sigmoid(x):
    return jax.nn.sigmoid(x)
def _layernorm(x, axis=-1, eps=1e-5):
    m = jnp.mean(x, axis=axis, keepdims=True)
    v = jnp.var(x, axis=axis, keepdims=True)
    return (x - m) / jnp.sqrt(v + eps)
def _scatter_add(tgt, idx, src, axis=0):
    return tgt.at[idx].add(src)
def _segment_sum(src, seg, n):
    return jax.ops.segment_sum(src, seg, n)
class _Rng:
    def __init__(self, key):
        self._k = key
    def _next(self):
        self._k, sub = jax.random.split(self._k)
        return sub
    def normal(self, shape):
        return jax.random.normal(self._next(), shape, dtype=jnp.bfloat16)
    def randint(self, lo, hi, shape):
        return jax.random.randint(self._next(), shape, lo, hi, dtype=jnp.int32)
    def uniform(self, shape, lo=0.0, hi=1.0):
        return jax.random.uniform(self._next(), shape, jnp.bfloat16, lo, hi)
    def permutation(self, n):
        return jax.random.permutation(self._next(), n)


kernel_name = 'gated_mix__mha_block__mixer_s_mlp__prompt'

def setup_inputs():
    _rng = _Rng(jax.random.key(int.from_bytes(__import__("os").urandom(4), "little")))
    _w = (lambda a: (lambda t: t.astype(jnp.bfloat16) if jnp.issubdtype(t.dtype, jnp.floating) else t)(jnp.asarray(a)))
    def _A_setup():
        B, S, D, H = 1, 2048, 512, 32
        return {
            "x": _w((lambda *s: _rng.normal(s) * 0.05)(B, S, D)),
            "wqkv": _w((lambda *s: _rng.normal(s) * 0.8)(D, 3 * D)),
            "wo": _w((lambda *s: _rng.normal(s) * 0.05)(D, D)),
        }
    _A_in = _A_setup()

    def _B_setup():
        B, S, D, F = 1, 2048, 512, 1792
        return {
            "x":  _w((lambda *s: _rng.normal(s) * 0.05)(B, S, D)),
            "w1": _w((lambda *s: _rng.normal(s) * 0.2)(D, D) * (D ** -0.5)),
            "w2": _w((lambda *s: _rng.normal(s) * 0.2)(D, D) * (D ** -0.5)),
            "w3": _w((lambda *s: _rng.normal(s) * 0.2)(D, F) * (D ** -0.5)),
            "w4": _w((lambda *s: _rng.normal(s) * 0.2)(F, D) * (F ** -0.5)),
        }
    _B_in = _B_setup()

    return {
        "A_x": _A_in["x"],
        "A_wqkv": _A_in["wqkv"],
        "A_wo": _A_in["wo"],
        "B_x": _B_in["x"],
        "B_w1": _B_in["w1"],
        "B_w2": _B_in["w2"],
        "B_w3": _B_in["w3"],
        "B_w4": _B_in["w4"],
        "gate_w": _w((lambda *s: _rng.normal(s) * 0.05)(512) * 16.0),
    }

def reference(A_x, A_wqkv, A_wo, B_x, B_w1, B_w2, B_w3, B_w4, gate_w):
    def _A_ref(x, wqkv, wo):
        B, S, D = x.shape
        H = 32
        Dh = D // H
        qkv = (lambda x, *d: x.transpose(*d))((x @ wqkv).reshape(B, S, 3, H, Dh), 2, 0, 3, 1, 4)
        q, k, v = qkv[0], qkv[1], qkv[2]
        scores = jnp.einsum("bhqd,bhkd->bhqk", q, k) * (Dh ** -0.5)
        p = _softmax(scores, axis=-1)
        o = jnp.einsum("bhqk,bhkd->bhqd", p, v)
        return (lambda x, *d: x.transpose(*d))(o, 0, 2, 1, 3).reshape(B, S, D) @ wo

    def _B_ref(x, w1, w2, w3, w4):
        B, S, D = x.shape
        h = _gelu(_layernorm(x, axis=-1) @ w1)
        c = D // 4
        g0 = jnp.pad(h[:, :, 0*c:1*c], ((0, 0), (1, 0), (0, 0)))[:, :S, :]
        g1 = jnp.pad(h[:, :, 1*c:2*c], ((0, 0), (0, 1), (0, 0)))[:, 1:, :]
        g2 = jnp.pad(h[:, :, 2*c:3*c], ((0, 0), (2, 0), (0, 0)))[:, :S, :]
        g3 = jnp.pad(h[:, :, 3*c:   ], ((0, 0), (0, 2), (0, 0)))[:, 2:, :]
        hs = jnp.concatenate([g0, g1, g2, g3], axis=-1) @ w2
        x1 = x + hs
        h2 = _gelu(_layernorm(x1, axis=-1) @ w3) @ w4
        return x1 + h2

    x = A_x
    g = _sigmoid((x * gate_w).sum(-1, keepdims=True))
    a = _A_ref(x, A_wqkv, A_wo)
    b = _B_ref(x, B_w1, B_w2, B_w3, B_w4)
    return g * a + (1 - g) * b
```

```python
import math

import jax
import jax.numpy as jnp
from jax.experimental import pallas as pl
from jax.experimental.pallas import tpu as pltpu

S = 2048
D = 512
H = 32
DH = 16
F = 1792
NG = D // 128
TQ = 512
TKJ = 128
NQ = S // TQ
NJ = S // TKJ
NITEM = H * NQ
UF = 4
LEAD = 2
LAG = 2
HPAD = 8
RB = 512
RC = 256
EPS = 1e-5
QSCALE = (DH ** -0.5) * math.log2(math.e)
L_LO = 2.0 ** -80
L_HI = 2.0 ** 126
O_HI = 3.0e38

bf16 = jnp.bfloat16
f32 = jnp.float32
i32 = jnp.int32


def _gelu(x):
    c = math.sqrt(2.0 / math.pi)
    return 0.5 * x * (1.0 + jnp.tanh(c * (x + 0.044715 * (x * x * x))))


def _layernorm(x):
    m = jnp.mean(x, axis=-1, keepdims=True)
    xc = x - m
    v = jnp.mean(xc * xc, axis=-1, keepdims=True)
    return xc * jax.lax.rsqrt(v + EPS)


def _dot(a, b):
    return jnp.dot(a, b, preferred_element_type=f32)


def _dot_nt(a, b):
    return jax.lax.dot_general(a, b, (((1,), (1,)), ((), ())), preferred_element_type=f32)


def _dot_tn(a, b):
    return jax.lax.dot_general(a, b, (((0,), (0,)), ((), ())), preferred_element_type=f32)


def _kernel(ax_hbm, wqkv_hbm, wo_hbm, w1_hbm, w2_hbm, w3_hbm, w4_hbm, gw_hbm,
            out_hbm,
            ax_s, wqkv_s, wo_s, w1_s, w2_s, w3_s, w4_s, gw_s,
            wqvt_s, k_s, qt_s, vt_s, ot_s, h_s, buf0, buf1, pbuf, obuf,
            in_sems, out_sems):
    nb = S // RB

    def ax_copy(i):
        return pltpu.make_async_copy(ax_hbm.at[0, pl.ds(i * RB, RB), :],
                                     ax_s.at[pl.ds(i * RB, RB), :], in_sems.at[i])

    w_copies = {}
    for n, (name, src, dst) in enumerate((
            ("w1", w1_hbm, w1_s), ("wqkv", wqkv_hbm, wqkv_s), ("w2", w2_hbm, w2_s),
            ("w3", w3_hbm, w3_s), ("w4", w4_hbm, w4_s), ("wo", wo_hbm, wo_s),
            ("gw", gw_hbm, gw_s))):
        w_copies[name] = pltpu.make_async_copy(src, dst, in_sems.at[nb + n])

    w_copies["w1"].start()
    for i in range(nb):
        ax_copy(i).start()
    w_copies["wqkv"].start()
    for name in ("w2", "w3", "w4", "wo", "gw"):
        w_copies[name].start()

    for g in range(NG):
        h_s[g, 0:HPAD, :] = jnp.zeros((HPAD, 128), f32)
        h_s[g, HPAD + S:HPAD + S + HPAD, :] = jnp.zeros((HPAD, 128), f32)
    w_copies["w1"].wait()
    for i in range(nb):
        ax_copy(i).wait()
        xb = ax_s[i * RB:(i + 1) * RB, :].astype(f32)
        h = _gelu(_dot(_layernorm(xb).astype(bf16), w1_s[...]))
        for g in range(NG):
            h_s[g, HPAD + i * RB:HPAD + (i + 1) * RB, :] = h[:, g * 128:(g + 1) * 128]

    w_copies["wqkv"].wait()
    for name in ("w2", "w3", "w4", "wo", "gw"):
        w_copies[name].wait()
    wqvt_s[0:D, :] = wqkv_s[:, 0:D].astype(f32).T.astype(bf16)
    wqvt_s[D:2 * D, :] = wqkv_s[:, 2 * D:3 * D].astype(f32).T.astype(bf16)
    for i in range(nb):
        xb = ax_s[i * RB:(i + 1) * RB, :]
        kb = _dot(xb, wqkv_s[:, D:2 * D]).astype(bf16)
        for g in range(NG):
            k_s[g, i * RB:(i + 1) * RB, :] = kb[:, g * 128:(g + 1) * 128]
        qv = _dot_nt(wqvt_s[...], xb)
        qt_s[:, i * RB:(i + 1) * RB] = (qv[0:D] * QSCALE).astype(bf16)
        vt_s[:, i * RB:(i + 1) * RB] = qv[D:2 * D].astype(bf16)

    def build_w(idx):
        h = idx // NQ
        qt = idx % NQ
        g = h // 8
        hl = h % 8
        qoff = pl.multiple_of(qt * TQ, TQ)
        qT = qt_s[pl.ds(pl.multiple_of(g * 128, 128), 128), pl.ds(qoff, TQ)]
        rows = jax.lax.broadcasted_iota(i32, (128, TQ), 0)
        return jnp.where((rows // DH) == hl, qT, jnp.zeros_like(qT)), g

    def f_scores(j, W, g, l8):
        p = jnp.exp2(_dot(k_s[g, j * TKJ:(j + 1) * TKJ, :], W))
        ps = jnp.sum(p.reshape(TKJ // 8, 8, TQ), axis=0)
        return p.astype(bf16), (ps if l8 is None else l8 + ps)

    def f_body(b, carry):
        bad, l8_carry = carry
        base = UF * b
        pq = [pbuf[i] for i in range(LEAD)]
        l8s = {0: l8_carry}
        W = None
        g = None
        acc = None
        for t in range(UF * NJ):
            u, j = divmod(t, NJ)
            au, aj = divmod(t + LEAD, NJ)
            if aj == 0 or W is None:
                W, g = build_w(jnp.minimum(base + au, NITEM - 1))
            pnew, l8s[au] = f_scores(aj, W, g, l8s.get(au) if aj > 0 else None)
            pq.append(pnew)
            item = base + u
            hoff = pl.multiple_of((item // NQ) * DH, DH)
            pv = _dot(vt_s[pl.ds(hoff, DH), j * TKJ:(j + 1) * TKJ], pq.pop(0))
            acc = pv if j == 0 else acc + pv
            if j == NJ - 1:
                qoff = pl.multiple_of((item % NQ) * TQ, TQ)
                l = jnp.sum(l8s[u], axis=0, keepdims=True)
                o = acc / l
                ok_l = jnp.logical_and(l >= L_LO, l <= L_HI)
                ok_o = jnp.abs(o) <= O_HI
                bad = jnp.maximum(bad, jnp.where(ok_l, 0.0, 1.0))
                bad = jnp.maximum(bad, jnp.max(jnp.where(ok_o, 0.0, 1.0), axis=0, keepdims=True))
                ot_s[pl.ds(hoff, DH), pl.ds(qoff, TQ)] = o.astype(bf16)
        for i in range(LEAD):
            pbuf[i] = pq[i]
        return bad, l8s[UF]

    W0, g0 = build_w(0)
    l80 = None
    for j in range(LEAD):
        p0, l80 = f_scores(j, W0, g0, l80)
        pbuf[j] = p0
    bad, _ = jax.lax.fori_loop(0, NITEM // UF, f_body, (jnp.zeros((1, TQ), f32), l80))

    def a_piece(j, W, g, buf, mx):
        s = _dot(k_s[g, j * TKJ:(j + 1) * TKJ, :], W)
        buf[j * TKJ:(j + 1) * TKJ, :] = s
        return jnp.maximum(mx, jnp.max(s.reshape(TKJ // 8, 8, TQ), axis=0))

    def b_piece(j, hoff, buf, m8, l8, acc):
        sc = buf[j * TKJ:(j + 1) * TKJ, :].reshape(TKJ // 8, 8, TQ)
        p = jnp.exp2(sc - m8[None])
        l8 = l8 + jnp.sum(p, axis=0)
        vt = vt_s[pl.ds(hoff, DH), j * TKJ:(j + 1) * TKJ]
        acc = acc + _dot(vt, p.reshape(TKJ, TQ).astype(bf16))
        return l8, acc

    def step(idx, m_cur, buf_cur, buf_nxt):
        W, g = build_w(jnp.minimum(idx + 1, NITEM - 1))
        hoff = pl.multiple_of((idx // NQ) * DH, DH)
        qoff = pl.multiple_of((idx % NQ) * TQ, TQ)
        mx = jnp.full((8, TQ), -jnp.inf, f32)
        l8 = jnp.zeros((8, TQ), f32)
        acc = jnp.zeros((DH, TQ), f32)
        zero = jnp.full((8, TQ), idx >> 24, i32)
        m8 = jnp.broadcast_to(m_cur, (8, TQ))
        m8i = pltpu.bitcast(m8, i32)
        hist = []
        for j in range(NJ):
            mx = a_piece(j, W, g, buf_nxt, mx)
            if len(hist) >= LAG:
                pmx, pl8 = hist[-LAG]
                dep = (pltpu.bitcast(pmx, i32) | pltpu.bitcast(pl8, i32)) & zero
                m_eff = pltpu.bitcast(m8i | dep, f32)
            else:
                m_eff = m8
            l8, acc = b_piece(j, hoff, buf_cur, m_eff, l8, acc)
            hist.append((mx, l8))
        l = jnp.sum(l8, axis=0, keepdims=True)
        ot_s[pl.ds(hoff, DH), pl.ds(qoff, TQ)] = (acc / l).astype(bf16)
        return jnp.max(mx, axis=0, keepdims=True)

    @pl.when(jnp.max(bad) > 0.0)
    def _():
        Ws, gs = build_w(0)
        mx0 = jnp.full((8, TQ), -jnp.inf, f32)
        for j in range(NJ):
            mx0 = a_piece(j, Ws, gs, buf0, mx0)
        m0 = jnp.max(mx0, axis=0, keepdims=True)

        def attn_body(i, m):
            m = step(2 * i, m, buf0, buf1)
            m = step(2 * i + 1, m, buf1, buf0)
            return m

        jax.lax.fori_loop(0, NITEM // 2, attn_body, m0)

    nc = S // RC

    def out_copy(i, slot):
        return pltpu.make_async_copy(obuf.at[slot], out_hbm.at[0, pl.ds(i * RC, RC), :],
                                     out_sems.at[slot])

    gwb = jnp.broadcast_to(gw_s[...], (128, D))
    for i in range(nc):
        r0 = i * RC
        slot = i % 2
        shifted = jnp.concatenate([
            h_s[0, HPAD + r0 - 1:HPAD + r0 - 1 + RC, :],
            h_s[1, HPAD + r0 + 1:HPAD + r0 + 1 + RC, :],
            h_s[2, HPAD + r0 - 2:HPAD + r0 - 2 + RC, :],
            h_s[3, HPAD + r0 + 2:HPAD + r0 + 2 + RC, :]], axis=-1)
        x1 = ax_s[r0:r0 + RC, :].astype(f32) + _dot(shifted.astype(bf16), w2_s[...])
        u = _gelu(_dot(_layernorm(x1).astype(bf16), w3_s[...]))
        b = x1 + _dot(u.astype(bf16), w4_s[...])
        a = _dot_tn(ot_s[:, r0:r0 + RC], wo_s[...])
        gate = jax.nn.sigmoid(_dot_nt(ax_s[r0:r0 + RC, :], gwb))
        gate = jnp.concatenate([gate] * NG, axis=-1)
        res = b + gate * (a - b)
        if i >= 2:
            out_copy(i - 2, slot).wait()
        obuf[slot] = res.astype(bf16)
        out_copy(i, slot).start()
    out_copy(nc - 2, (nc - 2) % 2).wait()
    out_copy(nc - 1, (nc - 1) % 2).wait()


@jax.jit
def pallas_gated_mix__mha_block__mixer_s_mlp__prompt_kernel(
    A_x: jax.Array,
    A_wqkv: jax.Array,
    A_wo: jax.Array,
    B_x: jax.Array,
    B_w1: jax.Array,
    B_w2: jax.Array,
    B_w3: jax.Array,
    B_w4: jax.Array,
    gate_w: jax.Array,
):
    nb = S // RB
    any_spec = pl.BlockSpec(memory_space=pl.ANY)
    return pl.pallas_call(
        _kernel,
        out_shape=jax.ShapeDtypeStruct((1, S, D), bf16),
        in_specs=[any_spec] * 8,
        out_specs=any_spec,
        scratch_shapes=[
            pltpu.VMEM((S, D), bf16),
            pltpu.VMEM((D, 3 * D), bf16),
            pltpu.VMEM((D, D), bf16),
            pltpu.VMEM((D, D), bf16),
            pltpu.VMEM((D, D), bf16),
            pltpu.VMEM((D, F), bf16),
            pltpu.VMEM((F, D), bf16),
            pltpu.VMEM((1, D), bf16),
            pltpu.VMEM((2 * D, D), bf16),
            pltpu.VMEM((NG, S, 128), bf16),
            pltpu.VMEM((D, S), bf16),
            pltpu.VMEM((D, S), bf16),
            pltpu.VMEM((D, S), bf16),
            pltpu.VMEM((NG, S + 2 * HPAD, 128), f32),
            pltpu.VMEM((S, TQ), f32),
            pltpu.VMEM((S, TQ), f32),
            pltpu.VMEM((LEAD, TKJ, TQ), bf16),
            pltpu.VMEM((2, RC, D), bf16),
            pltpu.SemaphoreType.DMA((nb + 7,)),
            pltpu.SemaphoreType.DMA((2,)),
        ],
        compiler_params=pltpu.CompilerParams(vmem_limit_bytes=100 * 1024 * 1024),
    )(A_x, A_wqkv, A_wo, B_w1, B_w2, B_w3, B_w4, gate_w.reshape(1, D))
```

```python
import math

import jax
import jax.numpy as jnp
from jax.experimental import pallas as pl
from jax.experimental.pallas import tpu as pltpu

S = 2048
D = 512
H = 32
DH = 16
F = 1792
NG = D // 128
TQ = 512
TKJ = 128
NQ = S // TQ
NJ = S // TKJ
NITEM = H * NQ
UF = 16
LEAD = 2
LAG = 2
HPAD = 8
RB = 512
RC = 256
EPS = 1e-5
QSCALE = (DH ** -0.5) * math.log2(math.e)
L_LO = 2.0 ** -80
L_HI = 2.0 ** 126
O_HI = 3.0e38

bf16 = jnp.bfloat16
f32 = jnp.float32
i32 = jnp.int32


def _gelu(x):
    c = math.sqrt(2.0 / math.pi)
    return 0.5 * x * (1.0 + jnp.tanh(c * (x + 0.044715 * (x * x * x))))


def _layernorm(x):
    m = jnp.mean(x, axis=-1, keepdims=True)
    xc = x - m
    v = jnp.mean(xc * xc, axis=-1, keepdims=True)
    return xc * jax.lax.rsqrt(v + EPS)


def _dot(a, b):
    return jnp.dot(a, b, preferred_element_type=f32)


def _dot_nt(a, b):
    return jax.lax.dot_general(a, b, (((1,), (1,)), ((), ())), preferred_element_type=f32)


def _dot_tn(a, b):
    return jax.lax.dot_general(a, b, (((0,), (0,)), ((), ())), preferred_element_type=f32)


def _kernel(ax_hbm, wqkv_hbm, wo_hbm, w1_hbm, w2_hbm, w3_hbm, w4_hbm, gw_hbm,
            out_hbm,
            ax_s, wqkv_s, wo_s, w1_s, w2_s, w3_s, w4_s, gw_s,
            wqvt_s, k_s, qt_s, vt_s, ot_s, h_s, buf0, buf1, pbuf, obuf,
            in_sems, out_sems):
    nb = S // RB

    def ax_copy(i):
        return pltpu.make_async_copy(ax_hbm.at[0, pl.ds(i * RB, RB), :],
                                     ax_s.at[pl.ds(i * RB, RB), :], in_sems.at[i])

    w_copies = {}
    for n, (name, src, dst) in enumerate((
            ("w1", w1_hbm, w1_s), ("wqkv", wqkv_hbm, wqkv_s), ("w2", w2_hbm, w2_s),
            ("w3", w3_hbm, w3_s), ("w4", w4_hbm, w4_s), ("wo", wo_hbm, wo_s),
            ("gw", gw_hbm, gw_s))):
        w_copies[name] = pltpu.make_async_copy(src, dst, in_sems.at[nb + n])

    w_copies["w1"].start()
    ax_copy(0).start()
    w_copies["wqkv"].start()
    for i in range(1, nb):
        ax_copy(i).start()
    for name in ("w2", "w3", "w4", "wo", "gw"):
        w_copies[name].start()

    def b1_block(i, nsub=1):
        rs = RB // nsub
        for c in range(nsub):
            r0 = i * RB + c * rs
            xb = ax_s[r0:r0 + rs, :].astype(f32)
            h = _gelu(_dot(_layernorm(xb).astype(bf16), w1_s[...]))
            for g in range(NG):
                h_s[g, HPAD + r0:HPAD + r0 + rs, :] = h[:, g * 128:(g + 1) * 128]

    def a1_k(i):
        kb = _dot(ax_s[i * RB:(i + 1) * RB, :], wqkv_s[:, D:2 * D]).astype(bf16)
        for g in range(NG):
            k_s[g, i * RB:(i + 1) * RB, :] = kb[:, g * 128:(g + 1) * 128]

    def a1_qv(i):
        qv = _dot_nt(wqvt_s[...], ax_s[i * RB:(i + 1) * RB, :])
        qt_s[:, i * RB:(i + 1) * RB] = (qv[0:D] * QSCALE).astype(bf16)
        vt_s[:, i * RB:(i + 1) * RB] = qv[D:2 * D].astype(bf16)

    for g in range(NG):
        h_s[g, 0:HPAD, :] = jnp.zeros((HPAD, 128), f32)
        h_s[g, HPAD + S:HPAD + S + HPAD, :] = jnp.zeros((HPAD, 128), f32)
    w_copies["w1"].wait()
    ax_copy(0).wait()
    b1_block(0, 4)
    w_copies["wqkv"].wait()
    ax_copy(1).wait()
    a1_k(0)
    wqvt_s[0:D, :] = wqkv_s[:, 0:D].astype(f32).T.astype(bf16)
    wqvt_s[D:2 * D, :] = wqkv_s[:, 2 * D:3 * D].astype(f32).T.astype(bf16)
    b1_block(1)
    a1_qv(0)
    for i in range(2, nb):
        ax_copy(i).wait()
    for i in range(1, nb):
        a1_k(i)
        if i + 1 < nb:
            b1_block(i + 1)
        a1_qv(i)

    def build_w(idx):
        h = idx // NQ
        qt = idx % NQ
        g = h // 8
        hl = h % 8
        qoff = pl.multiple_of(qt * TQ, TQ)
        qT = qt_s[pl.ds(pl.multiple_of(g * 128, 128), 128), pl.ds(qoff, TQ)]
        rows = jax.lax.broadcasted_iota(i32, (128, TQ), 0)
        return jnp.where((rows // DH) == hl, qT, jnp.zeros_like(qT)), g

    def f_scores(j, W, g, l8):
        p = jnp.exp2(_dot(k_s[g, j * TKJ:(j + 1) * TKJ, :], W))
        ps = jnp.sum(p.reshape(TKJ // 8, 8, TQ), axis=0)
        return p.astype(bf16), (ps if l8 is None else l8 + ps)

    def f_body(b, carry):
        bad, l8_carry = carry
        base = UF * b
        pq = [pbuf[i] for i in range(LEAD)]
        l8s = {0: l8_carry}
        W = None
        g = None
        acc = None
        for t in range(UF * NJ):
            u, j = divmod(t, NJ)
            au, aj = divmod(t + LEAD, NJ)
            if aj == 0 or W is None:
                W, g = build_w(jnp.minimum(base + au, NITEM - 1))
            pnew, l8s[au] = f_scores(aj, W, g, l8s.get(au) if aj > 0 else None)
            pq.append(pnew)
            item = base + u
            hoff = pl.multiple_of((item // NQ) * DH, DH)
            pv = _dot(vt_s[pl.ds(hoff, DH), j * TKJ:(j + 1) * TKJ], pq.pop(0))
            acc = pv if j == 0 else acc + pv
            if j == NJ - 1:
                qoff = pl.multiple_of((item % NQ) * TQ, TQ)
                l = jnp.sum(l8s[u], axis=0, keepdims=True)
                o = acc / l
                ok_l = jnp.logical_and(l >= L_LO, l <= L_HI)
                ok_o = jnp.abs(o) <= O_HI
                bad = jnp.maximum(bad, jnp.where(ok_l, 0.0, 1.0))
                bad = jnp.maximum(bad, jnp.max(jnp.where(ok_o, 0.0, 1.0), axis=0, keepdims=True))
                ot_s[pl.ds(hoff, DH), pl.ds(qoff, TQ)] = o.astype(bf16)
        for i in range(LEAD):
            pbuf[i] = pq[i]
        return bad, l8s[UF]

    W0, g0 = build_w(0)
    l80 = None
    for j in range(LEAD):
        p0, l80 = f_scores(j, W0, g0, l80)
        pbuf[j] = p0
    bad, _ = jax.lax.fori_loop(0, NITEM // UF, f_body, (jnp.zeros((1, TQ), f32), l80))

    def a_piece(j, W, g, buf, mx):
        s = _dot(k_s[g, j * TKJ:(j + 1) * TKJ, :], W)
        buf[j * TKJ:(j + 1) * TKJ, :] = s
        return jnp.maximum(mx, jnp.max(s.reshape(TKJ // 8, 8, TQ), axis=0))

    def b_piece(j, hoff, buf, m8, l8, acc):
        sc = buf[j * TKJ:(j + 1) * TKJ, :].reshape(TKJ // 8, 8, TQ)
        p = jnp.exp2(sc - m8[None])
        l8 = l8 + jnp.sum(p, axis=0)
        vt = vt_s[pl.ds(hoff, DH), j * TKJ:(j + 1) * TKJ]
        acc = acc + _dot(vt, p.reshape(TKJ, TQ).astype(bf16))
        return l8, acc

    def step(idx, m_cur, buf_cur, buf_nxt):
        W, g = build_w(jnp.minimum(idx + 1, NITEM - 1))
        hoff = pl.multiple_of((idx // NQ) * DH, DH)
        qoff = pl.multiple_of((idx % NQ) * TQ, TQ)
        mx = jnp.full((8, TQ), -jnp.inf, f32)
        l8 = jnp.zeros((8, TQ), f32)
        acc = jnp.zeros((DH, TQ), f32)
        zero = jnp.full((8, TQ), idx >> 24, i32)
        m8 = jnp.broadcast_to(m_cur, (8, TQ))
        m8i = pltpu.bitcast(m8, i32)
        hist = []
        for j in range(NJ):
            mx = a_piece(j, W, g, buf_nxt, mx)
            if len(hist) >= LAG:
                pmx, pl8 = hist[-LAG]
                dep = (pltpu.bitcast(pmx, i32) | pltpu.bitcast(pl8, i32)) & zero
                m_eff = pltpu.bitcast(m8i | dep, f32)
            else:
                m_eff = m8
            l8, acc = b_piece(j, hoff, buf_cur, m_eff, l8, acc)
            hist.append((mx, l8))
        l = jnp.sum(l8, axis=0, keepdims=True)
        ot_s[pl.ds(hoff, DH), pl.ds(qoff, TQ)] = (acc / l).astype(bf16)
        return jnp.max(mx, axis=0, keepdims=True)

    @pl.when(jnp.max(bad) > 0.0)
    def _():
        Ws, gs = build_w(0)
        mx0 = jnp.full((8, TQ), -jnp.inf, f32)
        for j in range(NJ):
            mx0 = a_piece(j, Ws, gs, buf0, mx0)
        m0 = jnp.max(mx0, axis=0, keepdims=True)

        def attn_body(i, m):
            m = step(2 * i, m, buf0, buf1)
            m = step(2 * i + 1, m, buf1, buf0)
            return m

        jax.lax.fori_loop(0, NITEM // 2, attn_body, m0)

    for name in ("w2", "w3", "w4", "wo", "gw"):
        w_copies[name].wait()
    blocks = [(r, RC) for r in range(0, S - RC, RC)]
    blocks += [(S - RC, RC // 2), (S - RC // 2, RC // 2)]
    nc = len(blocks)

    def out_copy(i):
        r0, rc = blocks[i]
        return pltpu.make_async_copy(obuf.at[pl.ds(r0, rc), :], out_hbm.at[0, pl.ds(r0, rc), :],
                                     out_sems.at[i])

    gw = gw_s[...].astype(f32).reshape(1, D)

    def mix_block(i):
        r0, rc = blocks[i]
        shifted = jnp.concatenate([
            h_s[0, HPAD + r0 - 1:HPAD + r0 - 1 + rc, :],
            h_s[1, HPAD + r0 + 1:HPAD + r0 + 1 + rc, :],
            h_s[2, HPAD + r0 - 2:HPAD + r0 - 2 + rc, :],
            h_s[3, HPAD + r0 + 2:HPAD + r0 + 2 + rc, :]], axis=-1)
        x = ax_s[r0:r0 + rc, :].astype(f32)
        gate = jax.nn.sigmoid(jnp.sum(x * gw, axis=-1, keepdims=True))
        x1 = x + _dot(shifted.astype(bf16), w2_s[...])
        return x1, _layernorm(x1).astype(bf16), gate

    nxt = mix_block(0)
    for i in range(nc):
        r0, rc = blocks[i]
        x1, xn, gate = nxt
        if i + 1 < nc:
            nxt = mix_block(i + 1)
        u = _gelu(_dot(xn, w3_s[...]))
        a = _dot_tn(ot_s[:, r0:r0 + rc], wo_s[...])
        b = x1 + _dot(u.astype(bf16), w4_s[...])
        res = b + gate * (a - b)
        obuf[r0:r0 + rc, :] = res.astype(bf16)
        out_copy(i).start()
    for i in range(nc):
        out_copy(i).wait()


@jax.jit
def pallas_gated_mix__mha_block__mixer_s_mlp__prompt_kernel(
    A_x: jax.Array,
    A_wqkv: jax.Array,
    A_wo: jax.Array,
    B_x: jax.Array,
    B_w1: jax.Array,
    B_w2: jax.Array,
    B_w3: jax.Array,
    B_w4: jax.Array,
    gate_w: jax.Array,
):
    nb = S // RB
    any_spec = pl.BlockSpec(memory_space=pl.ANY)
    return pl.pallas_call(
        _kernel,
        out_shape=jax.ShapeDtypeStruct((1, S, D), bf16),
        in_specs=[any_spec] * 8,
        out_specs=any_spec,
        scratch_shapes=[
            pltpu.VMEM((S, D), bf16),
            pltpu.VMEM((D, 3 * D), bf16),
            pltpu.VMEM((D, D), bf16),
            pltpu.VMEM((D, D), bf16),
            pltpu.VMEM((D, D), bf16),
            pltpu.VMEM((D, F), bf16),
            pltpu.VMEM((F, D), bf16),
            pltpu.VMEM((D,), bf16),
            pltpu.VMEM((2 * D, D), bf16),
            pltpu.VMEM((NG, S, 128), bf16),
            pltpu.VMEM((D, S), bf16),
            pltpu.VMEM((D, S), bf16),
            pltpu.VMEM((D, S), bf16),
            pltpu.VMEM((NG, S + 2 * HPAD, 128), f32),
            pltpu.VMEM((S, TQ), f32),
            pltpu.VMEM((S, TQ), f32),
            pltpu.VMEM((LEAD, TKJ, TQ), bf16),
            pltpu.VMEM((S, D), bf16),
            pltpu.SemaphoreType.DMA((nb + 7,)),
            pltpu.SemaphoreType.DMA((S // RC + 1,)),
        ],
        compiler_params=pltpu.CompilerParams(vmem_limit_bytes=100 * 1024 * 1024),
    )(A_x, A_wqkv, A_wo, B_w1, B_w2, B_w3, B_w4, gate_w)
```

```python
import math

import jax
import jax.numpy as jnp
from jax.experimental import pallas as pl
from jax.experimental.pallas import tpu as pltpu

S = 2048
D = 512
H = 32
DH = 16
F = 1792
NG = D // 128
TQ = 512
TKJ = 128
NQ = S // TQ
NJ = S // TKJ
NITEM = H * NQ
LEAD = 2
NV = 128
NM = (S - NV) // TKJ
NKG = NV // 8
KGC = 2
NL = TQ // 128
LAG = 2
HPAD = 8
RB = 512
RC = 256
EPS = 1e-5
QSCALE = (DH ** -0.5) * math.log2(math.e)
L_LO = 2.0 ** -80
L_HI = 2.0 ** 126
O_HI = 3.0e38

bf16 = jnp.bfloat16
f32 = jnp.float32
i32 = jnp.int32


def _gelu(x):
    c = math.sqrt(2.0 / math.pi)
    return 0.5 * x * (1.0 + jnp.tanh(c * (x + 0.044715 * (x * x * x))))


def _layernorm(x):
    m = jnp.mean(x, axis=-1, keepdims=True)
    xc = x - m
    v = jnp.mean(xc * xc, axis=-1, keepdims=True)
    return xc * jax.lax.rsqrt(v + EPS)


def _dot(a, b):
    return jnp.dot(a, b, preferred_element_type=f32)


def _dot_nt(a, b):
    return jax.lax.dot_general(a, b, (((1,), (1,)), ((), ())), preferred_element_type=f32)


def _dot_tn(a, b):
    return jax.lax.dot_general(a, b, (((0,), (0,)), ((), ())), preferred_element_type=f32)


def _kernel(ax_hbm, wqkv_hbm, wo_hbm, w1_hbm, w2_hbm, w3_hbm, w4_hbm, gw_hbm,
            out_hbm,
            ax_s, wqkv_s, wo_s, w1_s, w2_s, w3_s, w4_s, gw_s,
            wqvt_s, k_s, qt_s, vt_s, ot_s, h_s, buf0, buf1, pbuf, obuf,
            qtf_s, kr_s, kb0, kb1, pv0, pv1, qb0, qb1,
            in_sems, out_sems):
    nb = S // RB

    def ax_copy(i):
        return pltpu.make_async_copy(ax_hbm.at[0, pl.ds(i * RB, RB), :],
                                     ax_s.at[pl.ds(i * RB, RB), :], in_sems.at[i])

    w_copies = {}
    for n, (name, src, dst) in enumerate((
            ("w1", w1_hbm, w1_s), ("wqkv", wqkv_hbm, wqkv_s), ("w2", w2_hbm, w2_s),
            ("w3", w3_hbm, w3_s), ("w4", w4_hbm, w4_s), ("wo", wo_hbm, wo_s),
            ("gw", gw_hbm, gw_s))):
        w_copies[name] = pltpu.make_async_copy(src, dst, in_sems.at[nb + n])

    w_copies["w1"].start()
    ax_copy(0).start()
    w_copies["wqkv"].start()
    for i in range(1, nb):
        ax_copy(i).start()
    for name in ("w2", "w3", "w4", "wo", "gw"):
        w_copies[name].start()

    def b1_block(i, nsub=1):
        rs = RB // nsub
        for c in range(nsub):
            r0 = i * RB + c * rs
            xb = ax_s[r0:r0 + rs, :].astype(f32)
            h = _gelu(_dot(_layernorm(xb).astype(bf16), w1_s[...]))
            for g in range(NG):
                h_s[g, HPAD + r0:HPAD + r0 + rs, :] = h[:, g * 128:(g + 1) * 128]

    def a1_k(i):
        kb = _dot(ax_s[i * RB:(i + 1) * RB, :], wqkv_s[:, D:2 * D]).astype(bf16)
        for g in range(NG):
            k_s[g, i * RB:(i + 1) * RB, :] = kb[:, g * 128:(g + 1) * 128]
        if i == nb - 1:
            for g in range(NG):
                kt = kb[RB - NV:RB, g * 128:(g + 1) * 128].astype(f32)
                for hl in range(8):
                    kr_s[g * 8 + hl] = kt if hl == 0 else pltpu.roll(kt, 128 - hl * DH, 1)

    def a1_qv(i):
        qv = _dot_nt(wqvt_s[...], ax_s[i * RB:(i + 1) * RB, :])
        qs = (qv[0:D] * QSCALE).astype(bf16)
        qt_s[:, i * RB:(i + 1) * RB] = qs
        qtf_s[:, i * RB:(i + 1) * RB] = qs.astype(f32)
        vt_s[:, i * RB:(i + 1) * RB] = qv[D:2 * D].astype(bf16)

    for g in range(NG):
        h_s[g, 0:HPAD, :] = jnp.zeros((HPAD, 128), f32)
        h_s[g, HPAD + S:HPAD + S + HPAD, :] = jnp.zeros((HPAD, 128), f32)
    w_copies["w1"].wait()
    ax_copy(0).wait()
    b1_block(0, 4)
    w_copies["wqkv"].wait()
    ax_copy(1).wait()
    a1_k(0)
    wqvt_s[0:D, :] = wqkv_s[:, 0:D].astype(f32).T.astype(bf16)
    wqvt_s[D:2 * D, :] = wqkv_s[:, 2 * D:3 * D].astype(f32).T.astype(bf16)
    b1_block(1)
    a1_qv(0)
    for i in range(2, nb):
        ax_copy(i).wait()
    for i in range(1, nb):
        a1_k(i)
        if i + 1 < nb:
            b1_block(i + 1)
        a1_qv(i)

    def build_w(idx):
        h = idx // NQ
        qt = idx % NQ
        g = h // 8
        hl = h % 8
        qoff = pl.multiple_of(qt * TQ, TQ)
        qT = qt_s[pl.ds(pl.multiple_of(g * 128, 128), 128), pl.ds(qoff, TQ)]
        rows = jax.lax.broadcasted_iota(i32, (128, TQ), 0)
        return jnp.where((rows // DH) == hl, qT, jnp.zeros_like(qT)), g

    vwork = [(c, d, gg) for c in range(NKG // KGC) for d in range(DH) for gg in range(KGC)]
    vper = -(-len(vwork) // NM)
    kwork = [(d, kg) for d in range(DH) for kg in range(NKG)]
    kq = len(kwork) // NQ
    kper = -(-kq // NM)
    kbs = (kb0, kb1)
    pvs = (pv0, pv1)
    qbs = (qb0, qb1)

    def svreg(sv, m):
        return sv[(m // NL) * 8:(m // NL) * 8 + 8, (m % NL) * 128:(m % NL) * 128 + 128]

    def kb_entry(h, d, kg, kb, tie):
        src = kr_s[h, kg * 8:(kg + 1) * 8, :]
        if tie is not None:
            src = jnp.where(tie[0], src, tie[1])
        kb[d, kg * 8:(kg + 1) * 8, :] = jnp.broadcast_to(src[:, d:d + 1], (8, 128))

    def qb_half(h, qt, d8, qb, tie):
        blk = qtf_s[pl.ds(pl.multiple_of(h * DH + d8 * 8, 8), 8), qt * TQ:(qt + 1) * TQ]
        if tie is not None:
            blk = jnp.where(tie[0], blk, tie[1])
        for r in range(8):
            qb[d8 * 8 + r] = jnp.broadcast_to(blk[r:r + 1, :], (8, TQ))

    def f_body(b, carry):
        bad, l8_carry, l8v = carry
        base = 2 * NQ * b
        true = jnp.full((8, 128), b >> 24, i32) == 0
        true4 = jnp.full((8, TQ), b >> 24, i32) == 0
        pq = [pbuf[i] for i in range(LEAD)]
        l8s = {0: l8_carry}
        W = None
        g = None
        ai = LEAD
        for u in range(2 * NQ):
            hh, qt = divmod(u, NQ)
            hoff = pl.multiple_of((2 * b + hh) * DH, DH)
            kb_use = kbs[((u + 1) // NQ) % 2]
            qb_use = qbs[(u + 1) % 2]
            pv_dst = pvs[(u + 1) % 2]
            nhh, nqt = divmod(u + 2, NQ)
            nh = jnp.minimum(2 * b + nhh, H - 1)
            bhl, bq = divmod(u + 1 + NQ, NQ)
            bh = jnp.minimum(2 * b + bhl, H - 1)
            kw = kwork[bq * kq:(bq + 1) * kq]
            acc = None
            wi = 0
            ki = 0
            accs = {}
            l8v_new = None
            for t in range(NM):
                au, aj = divmod(ai, NM)
                ai += 1
                if aj == 0 or W is None:
                    W, g = build_w(jnp.minimum(base + au, NITEM - 1))
                sc = _dot(k_s[g, aj * TKJ:(aj + 1) * TKJ, :], W)
                p = jnp.exp2(sc)
                ps = jnp.sum(p.reshape(TKJ // 8, 8, TQ), axis=0)
                l8s[au] = ps if aj == 0 else l8s[au] + ps
                pq.append(p.astype(bf16))
                for n in range(vper):
                    if wi >= len(vwork):
                        break
                    c, d, gg = vwork[wi]
                    wi += 1
                    kg = c * KGC + gg
                    kbv = jnp.where(true, kb_use[d, kg * 8:(kg + 1) * 8, :], svreg(sc, (n * 64) // vper))
                    tt = jnp.concatenate([kbv] * NL, axis=1) * qb_use[d]
                    accs[gg] = tt if d == 0 else accs[gg] + tt
                    if d == DH - 1:
                        pf = jnp.exp2(accs[gg])
                        l8v_new = pf if l8v_new is None else l8v_new + pf
                        pv_dst[kg] = pf
                for n in range(kper):
                    if ki >= len(kw):
                        break
                    d, kg = kw[ki]
                    ki += 1
                    kb_entry(bh, d, kg, kbs[bhl % 2], (true, svreg(sc, (n * 64) // kper + 2)))
                if t in (2, 7):
                    qb_half(nh, nqt, 0 if t == 2 else 1, qbs[u % 2], (true4, sc[64:72, :]))
                pv = _dot(vt_s[pl.ds(hoff, DH), t * TKJ:(t + 1) * TKJ], pq.pop(0))
                acc = pv if acc is None else acc + pv
                if t == NM // 2:
                    pp = pvs[u % 2][...].reshape(NV, TQ).astype(bf16)
                    acc = acc + _dot(vt_s[pl.ds(hoff, DH), S - NV:S], pp)
            l = jnp.sum(l8s[u] + l8v, axis=0, keepdims=True)
            l8v = l8v_new
            o = acc / l
            ok_l = jnp.logical_and(l >= L_LO, l <= L_HI)
            ok_o = jnp.abs(o) <= O_HI
            bad = jnp.maximum(bad, jnp.where(ok_l, 0.0, 1.0))
            bad = jnp.maximum(bad, jnp.max(jnp.where(ok_o, 0.0, 1.0), axis=0, keepdims=True))
            ot_s[pl.ds(hoff, DH), qt * TQ:(qt + 1) * TQ] = o.astype(bf16)
        for i in range(LEAD):
            pbuf[i] = pq[i]
        return bad, l8s[2 * NQ], l8v

    for d, kg in kwork:
        kb_entry(0, d, kg, kb0, None)
    for d, kg in kwork[0:kq]:
        kb_entry(1, d, kg, kb1, None)
    for d8 in range(2):
        qb_half(0, 1, d8, qb1, None)
    W0, g0 = build_w(0)
    pf0 = jnp.exp2(_dot(k_s[g0, S - NV:S, :], W0)).reshape(NKG, 8, TQ)
    pv0[...] = pf0
    l8v0 = jnp.sum(pf0, axis=0)
    l80 = None
    for j in range(LEAD):
        p0 = jnp.exp2(_dot(k_s[g0, j * TKJ:(j + 1) * TKJ, :], W0))
        ps0 = jnp.sum(p0.reshape(TKJ // 8, 8, TQ), axis=0)
        l80 = ps0 if l80 is None else l80 + ps0
        pbuf[j] = p0.astype(bf16)
    bad, _, _ = jax.lax.fori_loop(0, H // 2, f_body, (jnp.zeros((1, TQ), f32), l80, l8v0))

    def a_piece(j, W, g, buf, mx):
        s = _dot(k_s[g, j * TKJ:(j + 1) * TKJ, :], W)
        buf[j * TKJ:(j + 1) * TKJ, :] = s
        return jnp.maximum(mx, jnp.max(s.reshape(TKJ // 8, 8, TQ), axis=0))

    def b_piece(j, hoff, buf, m8, l8, acc):
        sc = buf[j * TKJ:(j + 1) * TKJ, :].reshape(TKJ // 8, 8, TQ)
        p = jnp.exp2(sc - m8[None])
        l8 = l8 + jnp.sum(p, axis=0)
        vt = vt_s[pl.ds(hoff, DH), j * TKJ:(j + 1) * TKJ]
        acc = acc + _dot(vt, p.reshape(TKJ, TQ).astype(bf16))
        return l8, acc

    def step(idx, m_cur, buf_cur, buf_nxt):
        W, g = build_w(jnp.minimum(idx + 1, NITEM - 1))
        hoff = pl.multiple_of((idx // NQ) * DH, DH)
        qoff = pl.multiple_of((idx % NQ) * TQ, TQ)
        mx = jnp.full((8, TQ), -jnp.inf, f32)
        l8 = jnp.zeros((8, TQ), f32)
        acc = jnp.zeros((DH, TQ), f32)
        zero = jnp.full((8, TQ), idx >> 24, i32)
        m8 = jnp.broadcast_to(m_cur, (8, TQ))
        m8i = pltpu.bitcast(m8, i32)
        hist = []
        for j in range(NJ):
            mx = a_piece(j, W, g, buf_nxt, mx)
            if len(hist) >= LAG:
                pmx, pl8 = hist[-LAG]
                dep = (pltpu.bitcast(pmx, i32) | pltpu.bitcast(pl8, i32)) & zero
                m_eff = pltpu.bitcast(m8i | dep, f32)
            else:
                m_eff = m8
            l8, acc = b_piece(j, hoff, buf_cur, m_eff, l8, acc)
            hist.append((mx, l8))
        l = jnp.sum(l8, axis=0, keepdims=True)
        ot_s[pl.ds(hoff, DH), pl.ds(qoff, TQ)] = (acc / l).astype(bf16)
        return jnp.max(mx, axis=0, keepdims=True)

    @pl.when(jnp.max(bad) > 0.0)
    def _():
        Ws, gs = build_w(0)
        mx0 = jnp.full((8, TQ), -jnp.inf, f32)
        for j in range(NJ):
            mx0 = a_piece(j, Ws, gs, buf0, mx0)
        m0 = jnp.max(mx0, axis=0, keepdims=True)

        def attn_body(i, m):
            m = step(2 * i, m, buf0, buf1)
            m = step(2 * i + 1, m, buf1, buf0)
            return m

        jax.lax.fori_loop(0, NITEM // 2, attn_body, m0)

    for name in ("w2", "w3", "w4", "wo", "gw"):
        w_copies[name].wait()
    blocks = [(r, RC) for r in range(0, S - RC, RC)]
    blocks += [(S - RC, RC // 2), (S - RC // 2, RC // 2)]
    nc = len(blocks)

    def out_copy(i):
        r0, rc = blocks[i]
        return pltpu.make_async_copy(obuf.at[pl.ds(r0, rc), :], out_hbm.at[0, pl.ds(r0, rc), :],
                                     out_sems.at[i])

    gw = gw_s[...].astype(f32).reshape(1, D)

    def mix_block(i):
        r0, rc = blocks[i]
        shifted = jnp.concatenate([
            h_s[0, HPAD + r0 - 1:HPAD + r0 - 1 + rc, :],
            h_s[1, HPAD + r0 + 1:HPAD + r0 + 1 + rc, :],
            h_s[2, HPAD + r0 - 2:HPAD + r0 - 2 + rc, :],
            h_s[3, HPAD + r0 + 2:HPAD + r0 + 2 + rc, :]], axis=-1)
        x = ax_s[r0:r0 + rc, :].astype(f32)
        gate = jax.nn.sigmoid(jnp.sum(x * gw, axis=-1, keepdims=True))
        x1 = x + _dot(shifted.astype(bf16), w2_s[...])
        return x1, _layernorm(x1).astype(bf16), gate

    nxt = mix_block(0)
    for i in range(nc):
        r0, rc = blocks[i]
        x1, xn, gate = nxt
        if i + 1 < nc:
            nxt = mix_block(i + 1)
        u = _gelu(_dot(xn, w3_s[...]))
        a = _dot_tn(ot_s[:, r0:r0 + rc], wo_s[...])
        b = x1 + _dot(u.astype(bf16), w4_s[...])
        res = b + gate * (a - b)
        obuf[r0:r0 + rc, :] = res.astype(bf16)
        out_copy(i).start()
    for i in range(nc):
        out_copy(i).wait()


@jax.jit
def pallas_gated_mix__mha_block__mixer_s_mlp__prompt_kernel(
    A_x: jax.Array,
    A_wqkv: jax.Array,
    A_wo: jax.Array,
    B_x: jax.Array,
    B_w1: jax.Array,
    B_w2: jax.Array,
    B_w3: jax.Array,
    B_w4: jax.Array,
    gate_w: jax.Array,
):
    nb = S // RB
    any_spec = pl.BlockSpec(memory_space=pl.ANY)
    return pl.pallas_call(
        _kernel,
        out_shape=jax.ShapeDtypeStruct((1, S, D), bf16),
        in_specs=[any_spec] * 8,
        out_specs=any_spec,
        scratch_shapes=[
            pltpu.VMEM((S, D), bf16),
            pltpu.VMEM((D, 3 * D), bf16),
            pltpu.VMEM((D, D), bf16),
            pltpu.VMEM((D, D), bf16),
            pltpu.VMEM((D, D), bf16),
            pltpu.VMEM((D, F), bf16),
            pltpu.VMEM((F, D), bf16),
            pltpu.VMEM((D,), bf16),
            pltpu.VMEM((2 * D, D), bf16),
            pltpu.VMEM((NG, S, 128), bf16),
            pltpu.VMEM((D, S), bf16),
            pltpu.VMEM((D, S), bf16),
            pltpu.VMEM((D, S), bf16),
            pltpu.VMEM((NG, S + 2 * HPAD, 128), f32),
            pltpu.VMEM((S, TQ), f32),
            pltpu.VMEM((S, TQ), f32),
            pltpu.VMEM((LEAD, TKJ, TQ), bf16),
            pltpu.VMEM((S, D), bf16),
            pltpu.VMEM((D, S), f32),
            pltpu.VMEM((H, NV, 128), f32),
            pltpu.VMEM((DH, NV, 128), f32),
            pltpu.VMEM((DH, NV, 128), f32),
            pltpu.VMEM((NKG, 8, TQ), f32),
            pltpu.VMEM((NKG, 8, TQ), f32),
            pltpu.VMEM((DH, 8, TQ), f32),
            pltpu.VMEM((DH, 8, TQ), f32),
            pltpu.SemaphoreType.DMA((nb + 7,)),
            pltpu.SemaphoreType.DMA((S // RC + 1,)),
        ],
        compiler_params=pltpu.CompilerParams(vmem_limit_bytes=100 * 1024 * 1024),
    )(A_x, A_wqkv, A_wo, B_w1, B_w2, B_w3, B_w4, gate_w)
```

```python
import math

import jax
import jax.numpy as jnp
from jax.experimental import pallas as pl
from jax.experimental.pallas import tpu as pltpu

S = 2048
D = 512
H = 32
DH = 16
F = 1792
NG = D // 128
TQ = 512
TKJ = 128
NQ = S // TQ
NJ = S // TKJ
NITEM = H * NQ
LEAD = 2
NV = 128
NM = (S - NV) // TKJ
NKG = NV // 8
KGC = 2
NL = TQ // 128
HB = 2
LAG = 2
HPAD = 8
RB = 512
RC = 256
EPS = 1e-5
QSCALE = (DH ** -0.5) * math.log2(math.e)
L_LO = 2.0 ** -80
L_HI = 2.0 ** 126
O_HI = 3.0e38

bf16 = jnp.bfloat16
f32 = jnp.float32
i32 = jnp.int32


def _gelu(x):
    c = math.sqrt(2.0 / math.pi)
    return 0.5 * x * (1.0 + jnp.tanh(c * (x + 0.044715 * (x * x * x))))


def _layernorm(x):
    m = jnp.mean(x, axis=-1, keepdims=True)
    xc = x - m
    v = jnp.mean(xc * xc, axis=-1, keepdims=True)
    return xc * jax.lax.rsqrt(v + EPS)


def _dot(a, b):
    return jnp.dot(a, b, preferred_element_type=f32)


def _dot_nt(a, b):
    return jax.lax.dot_general(a, b, (((1,), (1,)), ((), ())), preferred_element_type=f32)


def _dot_tn(a, b):
    return jax.lax.dot_general(a, b, (((0,), (0,)), ((), ())), preferred_element_type=f32)


def _kernel(ax_hbm, wqkv_hbm, wo_hbm, w1_hbm, w2_hbm, w3_hbm, w4_hbm, gw_hbm,
            out_hbm,
            ax_s, wqkv_s, wo_s, w1_s, w2_s, w3_s, w4_s, gw_s,
            wqvt_s, k_s, qt_s, vt_s, ot_s, h_s, buf0, buf1, pbuf, obuf,
            qtf_s, kr_s, kb0, kb1, pv0, pv1, qb0, qb1,
            in_sems, out_sems):
    nb = S // RB

    def ax_copy(i):
        return pltpu.make_async_copy(ax_hbm.at[0, pl.ds(i * RB, RB), :],
                                     ax_s.at[pl.ds(i * RB, RB), :], in_sems.at[i])

    w_copies = {}
    for n, (name, src, dst) in enumerate((
            ("w1", w1_hbm, w1_s), ("wqkv", wqkv_hbm, wqkv_s), ("w2", w2_hbm, w2_s),
            ("w3", w3_hbm, w3_s), ("w4", w4_hbm, w4_s), ("wo", wo_hbm, wo_s),
            ("gw", gw_hbm, gw_s))):
        w_copies[name] = pltpu.make_async_copy(src, dst, in_sems.at[nb + n])

    w_copies["w1"].start()
    ax_copy(0).start()
    w_copies["wqkv"].start()
    for i in range(1, nb):
        ax_copy(i).start()
    for name in ("w2", "w3", "w4", "wo", "gw"):
        w_copies[name].start()

    def b1_block(i, nsub=1):
        rs = RB // nsub
        for c in range(nsub):
            r0 = i * RB + c * rs
            xb = ax_s[r0:r0 + rs, :].astype(f32)
            h = _gelu(_dot(_layernorm(xb).astype(bf16), w1_s[...]))
            for g in range(NG):
                h_s[g, HPAD + r0:HPAD + r0 + rs, :] = h[:, g * 128:(g + 1) * 128]

    def a1_k(i):
        kb = _dot(ax_s[i * RB:(i + 1) * RB, :], wqkv_s[:, D:2 * D]).astype(bf16)
        for g in range(NG):
            k_s[g, i * RB:(i + 1) * RB, :] = kb[:, g * 128:(g + 1) * 128]
        if i == nb - 1:
            for g in range(NG):
                kt = kb[RB - NV:RB, g * 128:(g + 1) * 128].astype(f32)
                for hl in range(8):
                    kr_s[g * 8 + hl] = kt if hl == 0 else pltpu.roll(kt, 128 - hl * DH, 1)

    def a1_qv(i):
        qv = _dot_nt(wqvt_s[...], ax_s[i * RB:(i + 1) * RB, :])
        qs = (qv[0:D] * QSCALE).astype(bf16)
        qt_s[:, i * RB:(i + 1) * RB] = qs
        qtf_s[:, i * RB:(i + 1) * RB] = qs.astype(f32)
        vt_s[:, i * RB:(i + 1) * RB] = qv[D:2 * D].astype(bf16)

    for g in range(NG):
        h_s[g, 0:HPAD, :] = jnp.zeros((HPAD, 128), f32)
        h_s[g, HPAD + S:HPAD + S + HPAD, :] = jnp.zeros((HPAD, 128), f32)
    w_copies["w1"].wait()
    ax_copy(0).wait()
    b1_block(0, 4)
    w_copies["wqkv"].wait()
    ax_copy(1).wait()
    a1_k(0)
    wqvt_s[0:D, :] = wqkv_s[:, 0:D].astype(f32).T.astype(bf16)
    wqvt_s[D:2 * D, :] = wqkv_s[:, 2 * D:3 * D].astype(f32).T.astype(bf16)
    b1_block(1)
    a1_qv(0)
    for i in range(2, nb):
        ax_copy(i).wait()
    for i in range(1, nb):
        a1_k(i)
        if i + 1 < nb:
            b1_block(i + 1)
        a1_qv(i)

    def build_w(idx):
        h = idx // NQ
        qt = idx % NQ
        g = h // 8
        hl = h % 8
        qoff = pl.multiple_of(qt * TQ, TQ)
        qT = qt_s[pl.ds(pl.multiple_of(g * 128, 128), 128), pl.ds(qoff, TQ)]
        rows = jax.lax.broadcasted_iota(i32, (128, TQ), 0)
        return jnp.where((rows // DH) == hl, qT, jnp.zeros_like(qT)), g

    vwork = [(c, d, gg) for c in range(NKG // KGC) for d in range(DH) for gg in range(KGC)]
    vper = -(-len(vwork) // NM)
    kwork = [(d, kg) for d in range(DH) for kg in range(NKG)]
    kq = len(kwork) // NQ
    kper = -(-kq // NM)
    kbs = (kb0, kb1)
    pvs = (pv0, pv1)
    qbs = (qb0, qb1)

    def svreg(sv, m):
        return sv[(m // NL) * 8:(m // NL) * 8 + 8, (m % NL) * 128:(m % NL) * 128 + 128]

    def kb_entry(h, d, kg, kb, tie):
        src = kr_s[h, kg * 8:(kg + 1) * 8, :]
        if tie is not None:
            src = jnp.where(tie[0], src, tie[1])
        kb[d, kg * 8:(kg + 1) * 8, :] = jnp.broadcast_to(src[:, d:d + 1], (8, 128))

    def qb_half(h, qt, d8, qb, tie):
        blk = qtf_s[pl.ds(pl.multiple_of(h * DH + d8 * 8, 8), 8), qt * TQ:(qt + 1) * TQ]
        if tie is not None:
            blk = jnp.where(tie[0], blk, tie[1])
        for r in range(8):
            qb[d8 * 8 + r] = jnp.broadcast_to(blk[r:r + 1, :], (8, TQ))

    def f_body(b, carry):
        bad, l8_carry, l8v = carry
        base = HB * NQ * b
        true = jnp.full((8, 128), b >> 24, i32) == 0
        true4 = jnp.full((8, TQ), b >> 24, i32) == 0
        pq = [pbuf[i] for i in range(LEAD)]
        l8s = {0: l8_carry}
        W = None
        g = None
        ai = LEAD
        for u in range(HB * NQ):
            hh, qt = divmod(u, NQ)
            hoff = pl.multiple_of((HB * b + hh) * DH, DH)
            kb_use = kbs[((u + 1) // NQ) % 2]
            qb_use = qbs[(u + 1) % 2]
            pv_dst = pvs[(u + 1) % 2]
            nhh, nqt = divmod(u + 2, NQ)
            nh = jnp.minimum(HB * b + nhh, H - 1)
            bhl, bq = divmod(u + 1 + NQ, NQ)
            bh = jnp.minimum(HB * b + bhl, H - 1)
            kw = kwork[bq * kq:(bq + 1) * kq]
            acc = None
            wi = 0
            ki = 0
            accs = {}
            l8v_new = None
            for t in range(NM):
                au, aj = divmod(ai, NM)
                ai += 1
                if aj == 0 or W is None:
                    W, g = build_w(jnp.minimum(base + au, NITEM - 1))
                sc = _dot(k_s[g, aj * TKJ:(aj + 1) * TKJ, :], W)
                p = jnp.exp2(sc)
                ps = jnp.sum(p.reshape(TKJ // 8, 8, TQ), axis=0)
                l8s[au] = ps if aj == 0 else l8s[au] + ps
                pq.append(p.astype(bf16))
                for n in range(vper):
                    if wi >= len(vwork):
                        break
                    c, d, gg = vwork[wi]
                    wi += 1
                    kg = c * KGC + gg
                    kbv = jnp.where(true, kb_use[d, kg * 8:(kg + 1) * 8, :], svreg(sc, (n * 64) // vper))
                    tt = jnp.concatenate([kbv] * NL, axis=1) * qb_use[d]
                    accs[gg] = tt if d == 0 else accs[gg] + tt
                    if d == DH - 1:
                        pf = jnp.exp2(accs[gg])
                        l8v_new = pf if l8v_new is None else l8v_new + pf
                        pv_dst[kg] = pf
                for n in range(kper):
                    if ki >= len(kw):
                        break
                    d, kg = kw[ki]
                    ki += 1
                    kb_entry(bh, d, kg, kbs[bhl % 2], (true, svreg(sc, (n * 64) // kper + 2)))
                if t in (2, 7):
                    qb_half(nh, nqt, 0 if t == 2 else 1, qbs[u % 2], (true4, sc[64:72, :]))
                pv = _dot(vt_s[pl.ds(hoff, DH), t * TKJ:(t + 1) * TKJ], pq.pop(0))
                acc = pv if acc is None else acc + pv
                if t == 0:
                    pp = pvs[u % 2][...].reshape(NV, TQ).astype(bf16)
                    acc = acc + _dot(vt_s[pl.ds(hoff, DH), S - NV:S], pp)
            l = jnp.sum(l8s[u] + l8v, axis=0, keepdims=True)
            l8v = l8v_new
            o = acc / l
            ok_l = jnp.logical_and(l >= L_LO, l <= L_HI)
            ok_o = jnp.abs(o) <= O_HI
            bad = jnp.maximum(bad, jnp.where(ok_l, 0.0, 1.0))
            bad = jnp.maximum(bad, jnp.max(jnp.where(ok_o, 0.0, 1.0), axis=0, keepdims=True))
            ot_s[pl.ds(hoff, DH), qt * TQ:(qt + 1) * TQ] = o.astype(bf16)
        for i in range(LEAD):
            pbuf[i] = pq[i]
        return bad, l8s[HB * NQ], l8v

    for d, kg in kwork:
        kb_entry(0, d, kg, kb0, None)
    for d, kg in kwork[0:kq]:
        kb_entry(1, d, kg, kb1, None)
    for d8 in range(2):
        qb_half(0, 1, d8, qb1, None)
    W0, g0 = build_w(0)
    pf0 = jnp.exp2(_dot(k_s[g0, S - NV:S, :], W0)).reshape(NKG, 8, TQ)
    pv0[...] = pf0
    l8v0 = jnp.sum(pf0, axis=0)
    l80 = None
    for j in range(LEAD):
        p0 = jnp.exp2(_dot(k_s[g0, j * TKJ:(j + 1) * TKJ, :], W0))
        ps0 = jnp.sum(p0.reshape(TKJ // 8, 8, TQ), axis=0)
        l80 = ps0 if l80 is None else l80 + ps0
        pbuf[j] = p0.astype(bf16)
    bad, _, _ = jax.lax.fori_loop(0, H // HB, f_body, (jnp.zeros((1, TQ), f32), l80, l8v0))

    def a_piece(j, W, g, buf, mx):
        s = _dot(k_s[g, j * TKJ:(j + 1) * TKJ, :], W)
        buf[j * TKJ:(j + 1) * TKJ, :] = s
        return jnp.maximum(mx, jnp.max(s.reshape(TKJ // 8, 8, TQ), axis=0))

    def b_piece(j, hoff, buf, m8, l8, acc):
        sc = buf[j * TKJ:(j + 1) * TKJ, :].reshape(TKJ // 8, 8, TQ)
        p = jnp.exp2(sc - m8[None])
        l8 = l8 + jnp.sum(p, axis=0)
        vt = vt_s[pl.ds(hoff, DH), j * TKJ:(j + 1) * TKJ]
        acc = acc + _dot(vt, p.reshape(TKJ, TQ).astype(bf16))
        return l8, acc

    def step(idx, m_cur, buf_cur, buf_nxt):
        W, g = build_w(jnp.minimum(idx + 1, NITEM - 1))
        hoff = pl.multiple_of((idx // NQ) * DH, DH)
        qoff = pl.multiple_of((idx % NQ) * TQ, TQ)
        mx = jnp.full((8, TQ), -jnp.inf, f32)
        l8 = jnp.zeros((8, TQ), f32)
        acc = jnp.zeros((DH, TQ), f32)
        zero = jnp.full((8, TQ), idx >> 24, i32)
        m8 = jnp.broadcast_to(m_cur, (8, TQ))
        m8i = pltpu.bitcast(m8, i32)
        hist = []
        for j in range(NJ):
            mx = a_piece(j, W, g, buf_nxt, mx)
            if len(hist) >= LAG:
                pmx, pl8 = hist[-LAG]
                dep = (pltpu.bitcast(pmx, i32) | pltpu.bitcast(pl8, i32)) & zero
                m_eff = pltpu.bitcast(m8i | dep, f32)
            else:
                m_eff = m8
            l8, acc = b_piece(j, hoff, buf_cur, m_eff, l8, acc)
            hist.append((mx, l8))
        l = jnp.sum(l8, axis=0, keepdims=True)
        ot_s[pl.ds(hoff, DH), pl.ds(qoff, TQ)] = (acc / l).astype(bf16)
        return jnp.max(mx, axis=0, keepdims=True)

    @pl.when(jnp.max(bad) > 0.0)
    def _():
        Ws, gs = build_w(0)
        mx0 = jnp.full((8, TQ), -jnp.inf, f32)
        for j in range(NJ):
            mx0 = a_piece(j, Ws, gs, buf0, mx0)
        m0 = jnp.max(mx0, axis=0, keepdims=True)

        def attn_body(i, m):
            m = step(2 * i, m, buf0, buf1)
            m = step(2 * i + 1, m, buf1, buf0)
            return m

        jax.lax.fori_loop(0, NITEM // 2, attn_body, m0)

    for name in ("w2", "w3", "w4", "wo", "gw"):
        w_copies[name].wait()
    blocks = [(r, RC) for r in range(0, S - RC, RC)]
    blocks += [(S - RC, RC // 2), (S - RC // 2, RC // 2)]
    nc = len(blocks)

    def out_copy(i):
        r0, rc = blocks[i]
        return pltpu.make_async_copy(obuf.at[pl.ds(r0, rc), :], out_hbm.at[0, pl.ds(r0, rc), :],
                                     out_sems.at[i])

    gw = gw_s[...].astype(f32).reshape(1, D)

    def mix_block(i):
        r0, rc = blocks[i]
        shifted = jnp.concatenate([
            h_s[0, HPAD + r0 - 1:HPAD + r0 - 1 + rc, :],
            h_s[1, HPAD + r0 + 1:HPAD + r0 + 1 + rc, :],
            h_s[2, HPAD + r0 - 2:HPAD + r0 - 2 + rc, :],
            h_s[3, HPAD + r0 + 2:HPAD + r0 + 2 + rc, :]], axis=-1)
        x = ax_s[r0:r0 + rc, :].astype(f32)
        gate = jax.nn.sigmoid(jnp.sum(x * gw, axis=-1, keepdims=True))
        x1 = x + _dot(shifted.astype(bf16), w2_s[...])
        return x1, _layernorm(x1).astype(bf16), gate

    nxt = mix_block(0)
    for i in range(nc):
        r0, rc = blocks[i]
        x1, xn, gate = nxt
        if i + 1 < nc:
            nxt = mix_block(i + 1)
        u = _gelu(_dot(xn, w3_s[...]))
        a = _dot_tn(ot_s[:, r0:r0 + rc], wo_s[...])
        b = x1 + _dot(u.astype(bf16), w4_s[...])
        res = b + gate * (a - b)
        obuf[r0:r0 + rc, :] = res.astype(bf16)
        out_copy(i).start()
    for i in range(nc):
        out_copy(i).wait()


@jax.jit
def pallas_gated_mix__mha_block__mixer_s_mlp__prompt_kernel(
    A_x: jax.Array,
    A_wqkv: jax.Array,
    A_wo: jax.Array,
    B_x: jax.Array,
    B_w1: jax.Array,
    B_w2: jax.Array,
    B_w3: jax.Array,
    B_w4: jax.Array,
    gate_w: jax.Array,
):
    nb = S // RB
    any_spec = pl.BlockSpec(memory_space=pl.ANY)
    return pl.pallas_call(
        _kernel,
        out_shape=jax.ShapeDtypeStruct((1, S, D), bf16),
        in_specs=[any_spec] * 8,
        out_specs=any_spec,
        scratch_shapes=[
            pltpu.VMEM((S, D), bf16),
            pltpu.VMEM((D, 3 * D), bf16),
            pltpu.VMEM((D, D), bf16),
            pltpu.VMEM((D, D), bf16),
            pltpu.VMEM((D, D), bf16),
            pltpu.VMEM((D, F), bf16),
            pltpu.VMEM((F, D), bf16),
            pltpu.VMEM((D,), bf16),
            pltpu.VMEM((2 * D, D), bf16),
            pltpu.VMEM((NG, S, 128), bf16),
            pltpu.VMEM((D, S), bf16),
            pltpu.VMEM((D, S), bf16),
            pltpu.VMEM((D, S), bf16),
            pltpu.VMEM((NG, S + 2 * HPAD, 128), f32),
            pltpu.VMEM((S, TQ), f32),
            pltpu.VMEM((S, TQ), f32),
            pltpu.VMEM((LEAD, TKJ, TQ), bf16),
            pltpu.VMEM((S, D), bf16),
            pltpu.VMEM((D, S), f32),
            pltpu.VMEM((H, NV, 128), f32),
            pltpu.VMEM((DH, NV, 128), f32),
            pltpu.VMEM((DH, NV, 128), f32),
            pltpu.VMEM((NKG, 8, TQ), f32),
            pltpu.VMEM((NKG, 8, TQ), f32),
            pltpu.VMEM((DH, 8, TQ), f32),
            pltpu.VMEM((DH, 8, TQ), f32),
            pltpu.SemaphoreType.DMA((nb + 7,)),
            pltpu.SemaphoreType.DMA((S // RC + 1,)),
        ],
        compiler_params=pltpu.CompilerParams(vmem_limit_bytes=100 * 1024 * 1024),
    )(A_x, A_wqkv, A_wo, B_w1, B_w2, B_w3, B_w4, gate_w)
```
